```python
import jax
import jax.numpy as jnp

def _softmax(x, axis=-1):
    return jax.nn.softmax(x, axis=axis)
def _gelu(x):
    return jax.nn.gelu(x, approximate=True)
def _silu(x):
    return jax.nn.silu(x)
def _sigmoid(x):
    return jax.nn.sigmoid(x)
def _layernorm(x, axis=-1, eps=1e-5):
    m = jnp.mean(x, axis=axis, keepdims=True)
    v = jnp.var(x, axis=axis, keepdims=True)
    return (x - m) / jnp.sqrt(v + eps)
def _scatter_add(tgt, idx, src, axis=0):
    return tgt.at[idx].add(src)
def _segment_sum(src, seg, n):
    return jax.ops.segment_sum(src, seg, n)
class _Rng:
    def __init__(self, key):
        self._k = key
    def _next(self):
        self._k, sub = jax.random.split(self._k)
        return sub
    def normal(self, shape):
        return jax.random.normal(self._next(), shape, dtype=jnp.bfloat16)
    def randint(self, lo, hi, shape):
        return jax.random.randint(self._next(), shape, lo, hi, dtype=jnp.int32)
    def uniform(self, shape, lo=0.0, hi=1.0):
        return jax.random.uniform(self._next(), shape, jnp.bfloat16, lo, hi)
    def permutation(self, n):
        return jax.random.permutation(self._next(), n)


kernel_name = 'interleave_layers__sliding_local_dilated__glu_gated_glu__prompt'

def setup_inputs():
    _rng = _Rng(jax.random.key(int.from_bytes(__import__("os").urandom(4), "little")))
    _w = (lambda a: (lambda t: t.astype(jnp.bfloat16) if jnp.issubdtype(t.dtype, jnp.floating) else t)(jnp.asarray(a)))
    def _A_setup():
        B, S, D = 1, 2048, 576
        return {
            "x": _w((lambda *s: _rng.normal(s) * 0.05)(B, S, D)),
            "wqkv": _w((lambda *s: _rng.normal(s) * 0.05)(D, 3 * D)),
            "wo": _w((lambda *s: _rng.normal(s) * 0.05)(D, D)),
        }
    _A_in = _A_setup()

    def _B_setup():
        B, S, D, F = 1, 2048, 576, 4608
        return {
            "x": _w((lambda *s: _rng.normal(s) * 0.05)(B, S, D)),
            "w_gate": _w((lambda *s: _rng.normal(s) * 0.05)(D, F)),
            "w_up": _w((lambda *s: _rng.normal(s) * 0.05)(D, F)),
            "w_down": _w((lambda *s: _rng.normal(s) * 0.05)(F, D)),
        }
    _B_in = _B_setup()

    return {
        "A_x": _A_in["x"],
        "A_wqkv": _A_in["wqkv"],
        "A_wo": _A_in["wo"],
        "B_x": _B_in["x"],
        "B_w_gate": _B_in["w_gate"],
        "B_w_up": _B_in["w_up"],
        "B_w_down": _B_in["w_down"],
    }

def reference(A_x, A_wqkv, A_wo, B_x, B_w_gate, B_w_up, B_w_down):
    def _A_ref(x, wqkv, wo):
        B, S, D = x.shape
        H = 32; Dh = D // H
        W, dil = 8, 2
        qkv = (lambda x, *d: x.transpose(*d))((x @ wqkv).reshape(B, S, 3, H, Dh), 2, 0, 3, 1, 4)
        q, k, v = qkv[0], qkv[1], qkv[2]
        scale = Dh ** -0.5
        pos = jnp.arange(S)
        off = jnp.arange(W) * dil
        idx = pos[:, None] - off[None, :]
        mask = idx >= 0
        idx_c = jnp.where(mask, idx, 0).reshape(-1)
        kg = k[:, :, idx_c, :].reshape(B, H, S, W, Dh)
        vg = v[:, :, idx_c, :].reshape(B, H, S, W, Dh)
        logits = jnp.einsum("bhsd,bhswd->bhsw", q, kg) * scale
        logits = jnp.where(mask[None, None, :, :], logits, -1e9)
        attn = _softmax(logits, axis=-1)
        o = jnp.einsum("bhsw,bhswd->bhsd", attn, vg)
        return (lambda x, *d: x.transpose(*d))(o, 0, 2, 1, 3).reshape(B, S, D) @ wo

    def _B_ref(x, w_gate, w_up, w_down):
        g = jnp.einsum("bsd,df->bsf", x, w_gate)
        u = jnp.einsum("bsd,df->bsf", x, w_up)
        h = _sigmoid(g) * u
        return jnp.einsum("bsf,fd->bsd", h, w_down)

    x = A_x
    x = x + _A_ref(_layernorm(x, axis=-1), A_wqkv, A_wo)
    x = x + _B_ref(_layernorm(x, axis=-1), B_w_gate, B_w_up, B_w_down)
    x = x + _A_ref(_layernorm(x, axis=-1), A_wqkv, A_wo)
    x = x + _B_ref(_layernorm(x, axis=-1), B_w_gate, B_w_up, B_w_down)
    return x
```

```python
import functools

import jax
import jax.numpy as jnp
import jax.experimental.pallas as pl
import jax.experimental.pallas.tpu as pltpu

S, D, F = 2048, 576, 4608
H, DH, W, DIL = 32, 18, 8, 2
LANES = 128
f32, bf16, u32 = jnp.float32, jnp.bfloat16, jnp.uint32


def _pack(x):
    return pltpu.bitcast(x.astype(bf16), u32)


def _unpack(x):
    return pltpu.bitcast(x, bf16)


def _gate(z):
    out = []
    for i in range(0, z.shape[0], 32):
        g, u = z[i:i + 16], z[i + 16:i + 32]
        out.append(u * jnp.tanh(g) + u)
    return jnp.concatenate(out, 0)


def _dot(a, b):
    return jnp.dot(a, b, preferred_element_type=f32)


def _layernorm_t(x):
    m = jnp.sum(x, axis=0, keepdims=True) * (1.0 / D)
    xc = x - m
    v = jnp.sum(xc * xc, axis=0, keepdims=True) * (1.0 / D)
    return xc * jax.lax.rsqrt(v + 1e-5)


def _lhs_combos(a11, a12, a21, a22):
    return [a11 + a22, a21 + a22, a11, a22, a11 + a12, a21 - a11, a12 - a22]


def _rhs_combos(b11, b12, b21, b22):
    return [b11 + b22, b11, b12 - b22, b21 - b11, b22, b11 + b12, b21 + b22]


def _combine(m):
    m1, m2, m3, m4, m5, m6, m7 = m
    return m1 + m4 - m5 + m7, m3 + m5, m2 + m4, m1 - m2 + m3 + m6


def make(ta=512, tb=256, fb=192, layers=2, do_a=True, do_b=True):
    nta = ta // LANES
    na = S // ta
    tm = 2 * tb
    ntb = tm // LANES
    nb = S // tm
    fu = 4 * fb
    nu = F // fu
    NT = S // LANES

    def kernel(x_hbm, wqkv_hbm, wo_hbm, wg_hbm, wu_hbm, wd_hbm, o_hbm,
               xio, xs, wqkv_raw, wo_raw, wg_raw, wu_raw, wd_raw,
               tmp, wqkv_t, wo_t, wp, wr, wd, halo, sem_x, sem_a, sem_f, sem_o):

        def x_copy(t):
            return pltpu.make_async_copy(x_hbm.at[:, pl.ds(t * LANES, LANES)], xio.at[t], sem_x.at[t])

        def o_copy(t):
            col = t * LANES if isinstance(t, int) else pl.multiple_of(t * LANES, LANES)
            return pltpu.make_async_copy(xio.at[t], o_hbm.at[:, pl.ds(col, LANES)], sem_o.at[t])

        def f_copies(c):
            return [pltpu.make_async_copy(src.at[:, pl.ds(c * fu, fu)], dst.at[c], sem_f.at[3 * c + i])
                    for i, (src, dst) in enumerate(((wg_hbm, wg_raw), (wu_hbm, wu_raw), (wd_hbm, wd_raw)))]

        qkv_copy = pltpu.make_async_copy(wqkv_hbm, wqkv_raw, sem_a.at[0])
        wo_copy = pltpu.make_async_copy(wo_hbm, wo_raw, sem_a.at[1])
        qkv_copy.start()
        for t in range(nta):
            x_copy(t).start()
        wo_copy.start()
        for t in range(nta, NT):
            x_copy(t).start()
        for c in range(nu):
            for cp in f_copies(c):
                cp.start()

        qkv_copy.wait()
        for kt in range(5):
            rows = min(LANES, D - kt * LANES)
            blk = wqkv_raw[kt * LANES:kt * LANES + rows, :].astype(f32)
            if rows < LANES:
                blk = jnp.concatenate([blk, jnp.zeros((LANES - rows, 3 * D), f32)], 0)
            tmp[kt] = blk.T
        for m in range(3):
            for hh in range(2):
                for d in range(DH):
                    r = m * D + hh * (D // 2) + d * 16
                    src = m * D + hh * (D // 2) + d
                    row = jnp.concatenate([tmp[kt, pl.ds(src, 16, stride=DH), :] for kt in range(5)], 1)
                    wqkv_t[r // 2:r // 2 + 8, :] = _pack(row)
        wo_copy.wait()
        wo32 = wo_raw[...].astype(f32)
        wo32 = jnp.concatenate([wo32, jnp.zeros((D, 5 * LANES - D), f32)], 1)
        for kt in range(5):
            tmp[kt, 0:D, :] = wo32[:, kt * LANES:(kt + 1) * LANES]
        rows = []
        for hh in range(2):
            for d in range(DH):
                src = hh * (D // 2) + d
                rows.append(jnp.concatenate([tmp[kt, pl.ds(src, 16, stride=DH), :] for kt in range(5)], 1).astype(bf16))
        rows.append(jnp.zeros((5 * LANES - D, 5 * LANES), bf16))
        wo_t[...] = _pack(jnp.concatenate(rows, 0).T)

        def prep_unit(c):
            for i, raw in enumerate((wg_raw, wu_raw)):
                p = raw[c, :, 0:2 * fb]
                q = raw[c, :, 2 * fb:4 * fb]
                pb, qb = p[448:512], q[448:512]
                pa, qa = p[512:576], q[512:576]
                pm = jnp.concatenate([p[0:448], (pb.astype(f32) - qb.astype(f32)).astype(bf16)], 0).T
                qm = jnp.concatenate([q[0:448], (qa.astype(f32) - pa.astype(f32)).astype(bf16)], 0).T
                rt = jnp.concatenate([qb, pa], 0).T
                rt = _pack(rt)
                for n in range(2 * fb // 16):
                    wr[c, 16 * n + 8 * i:16 * n + 8 * i + 8, :] = rt[8 * n:8 * n + 8]
                for s, mt in enumerate((pm, qm)):
                    mt = mt.astype(f32)
                    combos = _lhs_combos(mt[:fb, :256], mt[:fb, 256:], mt[fb:, :256], mt[fb:, 256:])
                    for j in range(7):
                        cj = _pack(combos[j])
                        for n in range(fb // 16):
                            wp[c, s, j, 16 * n + 8 * i:16 * n + 8 * i + 8, :] = cj[8 * n:8 * n + 8]
            dt = wd_raw[c].astype(f32)
            hd = D // 2
            combos = _lhs_combos(dt[:hd, :2 * fb], dt[:hd, 2 * fb:], dt[hd:, :2 * fb], dt[hd:, 2 * fb:])
            for j in range(7):
                wd[c, j] = _pack(combos[j])

        def attn_block(i):
            t0 = i * nta
            x = jnp.concatenate([xs[t0 + j] for j in range(nta)], 1)
            xn = _layernorm_t(x).astype(bf16)
            lane8 = jax.lax.broadcasted_iota(jnp.int32, (8, LANES), 1)
            lane16 = jax.lax.broadcasted_iota(jnp.int32, (16, LANES), 1)
            qkv = _dot(_unpack(wqkv_t[:, 0:D]), xn)
            k = pltpu.bitcast(qkv[D:2 * D].astype(bf16), jnp.uint32)
            v = pltpu.bitcast(qkv[2 * D:].astype(bf16), jnp.uint32)
            kprev, vprev = halo[0], halo[1]
            o_tiles = []
            for j in range(nta):
                cols = slice(j * LANES, (j + 1) * LANES)
                kcur, vcur = k[:, cols], v[:, cols]

                def shifted(prev, cur, w):
                    if w:
                        cur = pltpu.roll(jnp.where(lane8 >= LANES - DIL * w, prev, cur), DIL * w, 1)
                    return pltpu.bitcast(cur, bf16).astype(f32)

                pos = lane16 + (t0 + j) * LANES
                o_rows = []
                for hh in range(2):
                    logits = [None] * W
                    for d in range(DH):
                        r = hh * DH + d
                        qd = qkv[16 * r:16 * r + 16, cols]
                        for w in range(W):
                            t = qd * shifted(kprev[8 * r:8 * r + 8], kcur[8 * r:8 * r + 8], w)
                            logits[w] = t if d == 0 else logits[w] + t
                    logits = [lg * (DH ** -0.5) for lg in logits]
                    if j == 0:
                        logits = [lg if w == 0 else jnp.where(pos >= DIL * w, lg, -1e9) for w, lg in enumerate(logits)]
                    mx = functools.reduce(jnp.maximum, logits)
                    e = [jnp.exp(lg - mx) for lg in logits]
                    inv = 1.0 / functools.reduce(lambda a, b: a + b, e)
                    p = [ew * inv for ew in e]
                    for d in range(DH):
                        r = hh * DH + d
                        acc = None
                        for w in range(W):
                            t = p[w] * shifted(vprev[8 * r:8 * r + 8], vcur[8 * r:8 * r + 8], w)
                            acc = t if w == 0 else acc + t
                        o_rows.append(acc.astype(bf16))
                o_tiles.append(jnp.concatenate(o_rows, 0))
                kprev, vprev = kcur, vcur
            halo[0] = kprev
            halo[1] = vprev
            y = x + _dot(_unpack(wo_t[0:D // 2, 0:D]), jnp.concatenate(o_tiles, 1))
            for j in range(nta):
                xs[t0 + j] = y[:, j * LANES:(j + 1) * LANES]

        def ffn_block(i):
            t0 = i * ntb
            x = jnp.concatenate([xs[t0 + j] for j in range(ntb)], 1)
            xn = _layernorm_t(x) * 0.5
            k1 = xn[0:256]
            xr = xn[448:576].astype(bf16)
            xc = []
            for k2 in (xn[256:512], jnp.concatenate([xn[256:448], xn[512:576]], 0)):
                xc.append([t.astype(bf16) for t in _rhs_combos(k1[:, :tb], k1[:, tb:], k2[:, :tb], k2[:, tb:])])
            acc = [None] * 7
            for c in range(nu):
                r = _dot(_unpack(wr[c]), xr)
                hs = []
                for s in range(2):
                    mm = lambda j: _dot(_unpack(wp[c, s, j - 1]), xc[s][j - 1])
                    m3, m5 = mm(3), mm(5)
                    h12 = _gate(r[:2 * fb, tb:] + m3 + m5)
                    m2, m4 = mm(2), mm(4)
                    h21 = _gate(r[2 * fb:, :tb] + m2 + m4)
                    t11 = r[:2 * fb, :tb] - m5 + m4
                    t22 = r[2 * fb:, tb:] + m3 - m2
                    m7, m1 = mm(7), mm(1)
                    h11 = _gate(t11 + m7 + m1)
                    h22 = _gate(t22 + m1 + mm(6))
                    hs += [jnp.concatenate([h11, h21], 0), jnp.concatenate([h12, h22], 0)]
                hc = _rhs_combos(*hs)
                for j in (1, 5, 3, 2, 4, 6, 0):
                    t = _dot(_unpack(wd[c, j]), hc[j].astype(bf16))
                    acc[j] = t if c == 0 else acc[j] + t
            o11, o12, o21, o22 = _combine(acc)
            y = x + jnp.concatenate([jnp.concatenate([o11, o12], 1), jnp.concatenate([o21, o22], 1)], 0)
            for j in range(ntb):
                yt = y[:, j * LANES:(j + 1) * LANES]
                xs[t0 + j] = yt
                xio[t0 + j] = yt.astype(bf16)

        for t in range(NT):
            x_copy(t).wait()
            xs[t] = xio[t].astype(f32)

        def layer(l, _):
            halo[...] = jnp.zeros(halo.shape, halo.dtype)
            if do_a:
                jax.lax.fori_loop(0, na, lambda i, _: attn_block(i), None)

            @pl.when(l == 0)
            def _():
                for c in range(nu):
                    for cp in f_copies(c):
                        cp.wait()
                jax.lax.fori_loop(0, nu, lambda c, _: prep_unit(c), None)

            def ffn_step(i, _):
                if do_b:
                    ffn_block(i)

                @pl.when(l == layers - 1)
                def _():
                    for j in range(ntb):
                        o_copy(i * ntb + j).start()

            jax.lax.fori_loop(0, nb, ffn_step, None)

        jax.lax.fori_loop(0, layers, layer, None)
        for t in range(NT):
            o_copy(t).wait()

    @jax.jit
    def f(A_x, A_wqkv, A_wo, B_x, B_w_gate, B_w_up, B_w_down):
        del B_x
        hbm = pl.BlockSpec(memory_space=pltpu.HBM)
        out = pl.pallas_call(
            kernel,
            out_shape=jax.ShapeDtypeStruct((D, S), bf16),
            in_specs=[hbm] * 6,
            out_specs=hbm,
            scratch_shapes=[
                pltpu.VMEM((NT, D, LANES), bf16),
                pltpu.VMEM((NT, D, LANES), f32),
                pltpu.VMEM((D, 3 * D), bf16),
                pltpu.VMEM((D, D), bf16),
                pltpu.VMEM((nu, D, fu), bf16),
                pltpu.VMEM((nu, D, fu), bf16),
                pltpu.VMEM((nu, D, fu), bf16),
                pltpu.VMEM((5, 3 * D, LANES), f32),
                pltpu.VMEM((3 * D // 2, 5 * LANES), u32),
                pltpu.VMEM((5 * LANES // 2, 5 * LANES), u32),
                pltpu.VMEM((nu, 2, 7, fb, 256), u32),
                pltpu.VMEM((nu, 2 * fb, LANES), u32),
                pltpu.VMEM((nu, 7, D // 4, 2 * fb), u32),
                pltpu.VMEM((2, D // 2, LANES), jnp.uint32),
                pltpu.SemaphoreType.DMA((NT,)),
                pltpu.SemaphoreType.DMA((2,)),
                pltpu.SemaphoreType.DMA((3 * nu,)),
                pltpu.SemaphoreType.DMA((NT,)),
            ],
            compiler_params=pltpu.CompilerParams(vmem_limit_bytes=120 * 2**20),
        )(A_x[0].T, A_wqkv, A_wo, B_w_gate, B_w_up, B_w_down.T)
        return out.T[None]

    return f


pallas_interleave_layers__sliding_local_dilated__glu_gated_glu__prompt_kernel = make(tb=128)
```

```python
import functools

import jax
import jax.numpy as jnp
import jax.experimental.pallas as pl
import jax.experimental.pallas.tpu as pltpu

S, D, F = 2048, 576, 4608
H, DH, W, DIL = 32, 18, 8, 2
HD = D // 2
LANES = 128
NT = S // LANES
BT = 4
NB = NT // BT
FP = 512
NP = F // FP
KROWS = (0, 128, 256, 384, 448)
f32, bf16, u32 = jnp.float32, jnp.bfloat16, jnp.uint32


def _half(words):
    return pltpu.bitcast(words, bf16)


def _dot(a, b):
    return jnp.dot(a, b, preferred_element_type=f32)


def _layernorm_t(x, scale=1.0):
    m = jnp.sum(x, axis=0, keepdims=True) * (1.0 / D)
    xc = x - m
    v = jnp.sum(xc * xc, axis=0, keepdims=True) * (1.0 / D)
    return xc * (jax.lax.rsqrt(v + 1e-5) * scale)


def _row_mean(load):
    parts = [load(r) for r in range(4)]
    for r in range(4, D // 8):
        parts[r % 4] = parts[r % 4] + load(r)
    total = jnp.sum((parts[0] + parts[1]) + (parts[2] + parts[3]), axis=0, keepdims=True)
    return total * (1.0 / D)


def _layernorm_coeffs(ref, t, scale):
    m = _row_mean(lambda r: ref[t, 8 * r:8 * r + 8, :])
    v = _row_mean(lambda r: jnp.square(ref[t, 8 * r:8 * r + 8, :] - m))
    a = jax.lax.rsqrt(v + 1e-5) * scale
    return jnp.broadcast_to(a, (16, LANES)), jnp.broadcast_to(m * a, (16, LANES))


def _gate(z):
    out = []
    for i in range(0, z.shape[0], 32):
        g, u = z[i:i + 16], z[i + 16:i + 32]
        out.append(u * jnp.tanh(g) + u)
    return jnp.concatenate(out, 0)


def _pair(p, q):
    low = jax.lax.broadcasted_iota(jnp.int32, p[0].shape, 1) < 64
    return (p[:3] + [jnp.where(low, p[3], p[3] - q[3])],
            q[:3] + [jnp.where(low, q[3], q[4] - p[4])],
            jnp.where(low, q[4], p[4]))


class _Quad:
    def __init__(self, v):
        self.v = list(v)

    def __add__(self, o):
        return _Quad(a + b for a, b in zip(self.v, o.v))

    def __sub__(self, o):
        return _Quad(a - b for a, b in zip(self.v, o.v))


def _quads(b):
    return [_Quad([b[2 * i][2 * j], b[2 * i][2 * j + 1], b[2 * i + 1][2 * j], b[2 * i + 1][2 * j + 1]])
            for i in range(2) for j in range(2)]


def _lhs_combo(n, a11, a12, a21, a22):
    return (lambda: a11 + a22, lambda: a21 + a22, lambda: a11, lambda: a22,
            lambda: a11 + a12, lambda: a21 - a11, lambda: a12 - a22)[n]()


def _rhs_combo(n, b11, b12, b21, b22):
    return (lambda: b11 + b22, lambda: b11, lambda: b12 - b22, lambda: b21 - b11,
            lambda: b22, lambda: b11 + b12, lambda: b21 + b22)[n]()


def _combos2(combo, blocks, emit):
    quads = _quads(blocks)
    for a in range(7):
        outer = combo(a, *quads)
        for b in range(7):
            emit(a, b, combo(b, *outer.v))


def _strassen(mm, fin, init=None):
    m3, m5 = mm(2), mm(4)
    fin(0, 1, m3 + m5 if init is None else init[1] + m3 + m5)
    m2, m4 = mm(1), mm(3)
    fin(1, 0, m2 + m4 if init is None else init[2] + m2 + m4)
    t11 = m4 - m5 if init is None else init[0] - m5 + m4
    t22 = m3 - m2 if init is None else init[3] + m3 - m2
    m7, m1 = mm(6), mm(0)
    fin(0, 0, t11 + m7 + m1)
    fin(1, 1, t22 + m1 + mm(5))


def _strassen2(mm, fin, init):
    def outer(a):
        out = [None] * 4

        def keep(i, j, v):
            out[2 * i + j] = v

        _strassen(lambda b: mm(a, b), keep)
        return _Quad(out)

    def fin_quad(i, j, quad):
        for n, v in enumerate(quad.v):
            fin(2 * i + n // 2, 2 * j + n % 2, v)

    _strassen(outer, fin_quad, _quads(init))


def make(n_early=3, group=3, layers=2, do_a=True, do_b=True, order="k01 q01 v01 S0 S1 k23 q23 P0 P1 N v23 S2 S3 o01 P2 P3 o23"):

    def kernel(x_hbm, wqkv_hbm, wo_hbm, wg_hbm, wu_hbm, wd_hbm, o_hbm,
               xio, xs, wqkv_raw, wo_raw, wg_raw, wu_raw, wd_raw,
               tmp, wa, wp, wr, wd, kv, xa, xc, xr, acc, ln, sem_x, sem_a, sem_f, sem_o):
        wa_w, wp_w, wr_w, wd_w, kv_w, xa_w, xc_w, xr_w = [t.bitcast(u32) for t in (wa, wp, wr, wd, kv, xa, xc, xr)]

        def aligned(i, n):
            return i * n if isinstance(i, int) else pl.multiple_of(i * n, n)

        def x_copy(t):
            return pltpu.make_async_copy(x_hbm.at[:, pl.ds(aligned(t, LANES), LANES)], xio.at[t], sem_x.at[t])

        def o_copy(t):
            return pltpu.make_async_copy(xio.at[t], o_hbm.at[:, pl.ds(aligned(t, LANES), LANES)], sem_o.at[t])

        def f_copies(n):
            return [pltpu.make_async_copy(src.at[:, pl.ds(aligned(n, FP), FP)], dst.at[n], sem_f.at[3 * n + i])
                    for i, (src, dst) in enumerate(((wg_hbm, wg_raw), (wu_hbm, wu_raw), (wd_hbm, wd_raw)))]

        def qkv_copy(c):
            rows = pl.ds(aligned(c, 64), 64)
            return pltpu.make_async_copy(wqkv_hbm.at[rows], wqkv_raw.at[rows], sem_a.at[c])

        wo_copy = pltpu.make_async_copy(wo_hbm, wo_raw, sem_a.at[9])

        def store_paired(m, row, p, q):
            p, q, r = _pair(p, q)
            for n, t in enumerate(p + q + [r]):
                wa[m, n, pl.ds(row, 16), :] = t.astype(bf16)

        def prep_wo():
            w32 = wo_raw[...].astype(f32)
            for n in range(5):
                c0 = min(n * LANES, D - LANES)
                tmp[n, 0:D, :] = w32[:, c0:c0 + LANES]
            tiles = []
            for n in range(5):
                rows = jnp.concatenate([tmp[n, pl.ds(hh * HD + d, 16, stride=DH), :]
                                        for hh in range(2) for d in range(DH)], 0).astype(bf16)
                tiles.append([rows[k0:k0 + LANES].T[(64 if n == 4 else 0):] for k0 in KROWS])
            full = [jnp.concatenate([t[k] for t in tiles], 0) for k in range(5)]
            for d in range(HD // 16):
                store_paired(3, 16 * d, [t[16 * d:16 * d + 16].astype(f32) for t in full],
                             [t[HD + 16 * d:HD + 16 * d + 16].astype(f32) for t in full])

        def transpose_qkv(kt, _):
            qkv_copy(2 * kt).wait()

            @pl.when(kt < 4)
            def _():
                qkv_copy(2 * kt + 1).wait()
            rows = pl.ds(pl.multiple_of(jnp.minimum(kt * LANES, D - LANES), 64), LANES)
            tmp[kt] = wqkv_raw[rows, :].T.astype(f32)

        def permute_qkv(m, _):
            for d in range(DH):
                p, q = [[tmp[k, pl.ds(m * D + hh * HD + d, 16, stride=DH), :] for k in range(5)] for hh in range(2)]
                store_paired(m, 16 * d, p, q)

        def prep_piece(n):
            tts = [[[raw[n, k0:k0 + LANES, i * LANES:(i + 1) * LANES].T for k0 in KROWS] for i in range(4)]
                   for raw in (wg_raw, wu_raw)]
            for r in range(9):
                blocks = [[wd_raw[n, 144 * i + 16 * r:144 * i + 16 * r + 16, k * LANES:(k + 1) * LANES].astype(f32)
                           for k in range(4)] for i in range(4)]

                def emit(a, b, v):
                    wd[n, a, b, 16 * r:16 * r + 16, :] = v.astype(bf16)
                _combos2(_lhs_combo, blocks, emit)
            for m, tt in enumerate(tts):
                for r in range(4):
                    row = 32 * r + 16 * m
                    paired = [_pair([t[16 * r:16 * r + 16].astype(f32) for t in tt[i]],
                                    [t[64 + 16 * r:64 + 16 * r + 16].astype(f32) for t in tt[i]]) for i in range(4)]
                    for i in range(4):
                        wr[n, 128 * i + row:128 * i + row + 16, :] = paired[i][2].astype(bf16)
                    for s in range(2):
                        def emit(a, b, v):
                            wp[n, s, a, b, row:row + 16, :] = v.astype(bf16)
                        _combos2(_lhs_combo, [t[s] for t in paired], emit)

        def attn_inputs(i):
            for j in range(BT):
                attn_input(j, i * BT + j)

        def attn_input(j, t):
            a, b = _layernorm_coeffs(xs, t, 1.0)
            for r in range(0, D, 16):
                xa[j, r:r + 16, :] = (xs[t, r:r + 16, :] * a - b).astype(bf16)

        def project(m, x):
            lhs = lambda lo, hi: _half(jnp.concatenate([wa_w[m, n] for n in range(lo, hi)], 1))
            r = _dot(lhs(8, 9), x[448:576])
            return (r + _dot(lhs(0, 4), x[0:512]),
                    r + _dot(lhs(4, 8), jnp.concatenate([x[0:448], x[512:576]], 0)))

        def attn_block(i):
            t0 = i * BT
            lane8 = jax.lax.broadcasted_iota(jnp.int32, (8, LANES), 1)
            lane16 = jax.lax.broadcasted_iota(jnp.int32, (16, LANES), 1)
            q, prob, o = {}, {}, {}

            def shifts(m, j, r):
                prev, cur = kv_w[m, j, 8 * r:8 * r + 8], kv_w[m, j + 1, 8 * r:8 * r + 8]
                out = [cur] + [pltpu.roll(jnp.where(lane8 >= LANES - DIL * w, prev, cur), DIL * w, 1)
                               for w in range(1, W)]
                return [_half(t).astype(f32) for t in out]

            def scores(j):
                for hh in range(2):
                    logits = None
                    for d in range(DH):
                        qd = q[j][hh][16 * d:16 * d + 16]
                        terms = [qd * t for t in shifts(0, j, hh * DH + d)]
                        logits = terms if d == 0 else [a + b for a, b in zip(logits, terms)]
                    logits = [t * (DH ** -0.5) for t in logits]
                    if j == 0:
                        pos = lane16 + t0 * LANES
                        logits = logits[:1] + [jnp.where(pos >= DIL * w, logits[w], -1e9) for w in range(1, W)]
                    mx = functools.reduce(jnp.maximum, logits)
                    e = [jnp.exp(t - mx) for t in logits]
                    inv = 1.0 / functools.reduce(jnp.add, e)
                    prob[j, hh] = [t * inv for t in e]

            def values(j):
                rows = []
                for hh in range(2):
                    for d in range(DH):
                        terms = [a * b for a, b in zip(prob[j, hh], shifts(1, j, hh * DH + d))]
                        rows.append(functools.reduce(jnp.add, terms))
                o[j] = jnp.concatenate(rows, 0).astype(bf16)

            for step in order.split():
                op, js = step[0], [int(c) for c in step[1:]]
                if op == "S":
                    scores(js[0])
                elif op == "P":
                    values(js[0])
                elif op == "N":
                    pass
                else:
                    m = "qkvo".index(op)
                    src = [o[j] if op == "o" else _half(xa_w[j]) for j in js]
                    halves = project(m, jnp.concatenate(src, 1))
                    for n, j in enumerate(js):
                        part = [t[:, n * LANES:(n + 1) * LANES] for t in halves]
                        if op == "q":
                            q[j] = part
                        for hh in range(2):
                            rows = slice(hh * HD, (hh + 1) * HD)
                            if op == "o":
                                xs[t0 + j, rows, :] += part[hh]
                            elif op != "q":
                                kv[m - 1, j + 1, rows, :] = part[hh].astype(bf16)
                if step == "v23":
                    attn_inputs(jnp.minimum(i + 1, NB - 1))
            for m in range(2):
                kv_w[m, 0] = kv_w[m, BT]

        def ffn_inputs(i):
            coeffs = [(ln[j, 0], ln[j, 1]) for j in range(BT)]
            for r in (4, 8, 5, 9, 6, 10, 7, 11, 0, 1, 2, 3):
                lo = 16 * (r if r < 8 else r - 4)
                blocks = [[xs[i * BT + j, k0:k0 + 16, :] * coeffs[j][0] - coeffs[j][1] for j in range(BT)]
                          for k0 in (lo, 128 + lo, 256 + lo, 384 + 16 * r)]
                if r >= 4:
                    for j in range(BT):
                        xr[j, 16 * r - 64:16 * r - 48, :] = blocks[3][j].astype(bf16)

                def emit(a, b, v):
                    xc[a, b, 16 * r:16 * r + 16, :] = v.astype(bf16)
                _combos2(_rhs_combo, blocks, emit)

        def ffn_stats(j, t):
            ln[j, 0], ln[j, 1] = _layernorm_coeffs(xs, t, 0.5)

        def ffn_block(i):
            t0 = i * BT
            hc = []
            ffn_inputs(i)
            shared = lambda n: _dot(_half(wr_w[n]), _half(jnp.concatenate([xr_w[j] for j in range(BT)], 1)))
            early = [shared(n) for n in range(n_early)]
            for n in range(NP):
                r = early[n] if n < n_early else shared(n)
                if n in (3, 4, 5, 6):
                    ffn_stats(n - 3, jnp.minimum(i + 1, NB - 1) * BT + n - 3)
                init = [[r[i * 128:(i + 1) * 128, j * LANES:(j + 1) * LANES] for j in range(4)] for i in range(4)]
                for s in range(2):
                    h = [[None] * 4 for _ in range(4)]

                    def mm(a, b):
                        rhs = jnp.concatenate([xc_w[a, b, 0:32], xc_w[a, b, 32 + 32 * s:64 + 32 * s]], 0)
                        return _dot(_half(wp_w[n, s, a, b]), _half(rhs))

                    def fin(i, j, v):
                        h[i][j] = _gate(v)
                    _strassen2(mm, fin, init)
                    combos = {}

                    def emit(a, b, v):
                        combos[a, b] = v.astype(bf16)
                    _combos2(_rhs_combo, h, emit)
                    hc.append(combos)
                if (n + 1) % group == 0:
                    def down(a, b):
                        lhs = jnp.concatenate([wd_w[m, a, b] for m in range(n + 1 - group, n + 1)], 1)
                        t = _dot(_half(lhs), jnp.concatenate([c[a, b] for c in hc], 0))
                        return t if n < group else acc[a, b] + t
                    if n < NP - 1:
                        for a in (1, 4, 2, 3, 5, 6, 0):
                            for b in range(7):
                                acc[a, b] = down(a, b)
                    else:
                        def out(i, j, v):
                            xs[t0 + j, 144 * i:144 * (i + 1), :] = v
                            xio[t0 + j, 144 * i:144 * (i + 1), :] = v.astype(bf16)
                        _strassen2(down, out, [[xs[t0 + j, 144 * i:144 * (i + 1), :] for j in range(4)] for i in range(4)])
                    hc = []

        def load_x(t, _):
            x_copy(t).wait()
            xs[t] = xio[t].astype(f32)

        wo_copy.start()
        for c in range(9):
            qkv_copy(c).start()
        wo_copy.wait()
        for t in range(NT):
            x_copy(t).start()
        prep_wo()
        jax.lax.fori_loop(0, 5, transpose_qkv, None)
        jax.lax.fori_loop(0, 3, permute_qkv, None)
        jax.lax.fori_loop(0, NT, load_x, None)
        for n in range(NP):
            for cp in f_copies(n):
                cp.start()

        def layer(l, _):
            for m in range(2):
                kv_w[m, 0] = jnp.zeros((HD, LANES), u32)
            def first_inputs(j, _):
                attn_input(j, j)
            jax.lax.fori_loop(0, BT, first_inputs, None)
            if do_a:
                jax.lax.fori_loop(0, NB, lambda i, _: attn_block(i), None)

            @pl.when(l == 0)
            def _():
                def step(n, _):
                    for cp in f_copies(n):
                        cp.wait()
                    prep_piece(n)
                jax.lax.fori_loop(0, NP, step, None)

            def ffn_step(i, _):
                if do_b:
                    ffn_block(i)

                @pl.when(l == layers - 1)
                def _():
                    for j in range(BT):
                        o_copy(i * BT + j).start()

            jax.lax.fori_loop(0, BT, lambda j, _: ffn_stats(j, j), None)
            jax.lax.fori_loop(0, NB, ffn_step, None)

        jax.lax.fori_loop(0, layers, layer, None)
        for t in range(NT):
            o_copy(t).wait()

    @jax.jit
    def f(A_x, A_wqkv, A_wo, B_x, B_w_gate, B_w_up, B_w_down):
        del B_x
        hbm = pl.BlockSpec(memory_space=pltpu.HBM)
        out = pl.pallas_call(
            kernel,
            out_shape=jax.ShapeDtypeStruct((D, S), bf16),
            in_specs=[hbm] * 6,
            out_specs=hbm,
            scratch_shapes=[
                pltpu.VMEM((NT, D, LANES), bf16),
                pltpu.VMEM((NT, D, LANES), f32),
                pltpu.VMEM((D, 3 * D), bf16),
                pltpu.VMEM((D, D), bf16),
                pltpu.VMEM((NP, D, FP), bf16),
                pltpu.VMEM((NP, D, FP), bf16),
                pltpu.VMEM((NP, D, FP), bf16),
                pltpu.VMEM((5, 3 * D, LANES), f32),
                pltpu.VMEM((4, 9, HD, LANES), bf16),
                pltpu.VMEM((NP, 2, 7, 7, 128, LANES), bf16),
                pltpu.VMEM((NP, 512, LANES), bf16),
                pltpu.VMEM((NP, 7, 7, 144, LANES), bf16),
                pltpu.VMEM((2, BT + 1, D, LANES), bf16),
                pltpu.VMEM((BT, D, LANES), bf16),
                pltpu.VMEM((7, 7, 192, LANES), bf16),
                pltpu.VMEM((BT, 128, LANES), bf16),
                pltpu.VMEM((7, 7, 144, LANES), f32),
                pltpu.VMEM((BT, 2, 16, LANES), f32),
                pltpu.SemaphoreType.DMA((NT,)),
                pltpu.SemaphoreType.DMA((10,)),
                pltpu.SemaphoreType.DMA((3 * NP,)),
                pltpu.SemaphoreType.DMA((NT,)),
            ],
            compiler_params=pltpu.CompilerParams(vmem_limit_bytes=120 * 2**20),
        )(A_x[0].T, A_wqkv, A_wo, B_w_gate, B_w_up, B_w_down.T)
        return out.T[None]

    return f


pallas_interleave_layers__sliding_local_dilated__glu_gated_glu__prompt_kernel = make()
```

```python
import functools

import jax
import jax.numpy as jnp
import jax.experimental.pallas as pl
import jax.experimental.pallas.tpu as pltpu

S, D, F = 2048, 576, 4608
H, DH, W, DIL = 32, 18, 8, 2
HD = D // 2
LANES = 128
NT = S // LANES
BT = 4
NB = NT // BT
FP = 512
NP = F // FP
KROWS = (0, 128, 256, 384, 448)
f32, bf16, u32 = jnp.float32, jnp.bfloat16, jnp.uint32


def _half(words):
    return pltpu.bitcast(words, bf16)


def _dot(a, b):
    return jnp.dot(a, b, preferred_element_type=f32)


def _layernorm_t(x, scale=1.0):
    m = jnp.sum(x, axis=0, keepdims=True) * (1.0 / D)
    xc = x - m
    v = jnp.sum(xc * xc, axis=0, keepdims=True) * (1.0 / D)
    return xc * (jax.lax.rsqrt(v + 1e-5) * scale)


def _row_mean(load):
    parts = [load(r) for r in range(4)]
    for r in range(4, D // 8):
        parts[r % 4] = parts[r % 4] + load(r)
    total = jnp.sum((parts[0] + parts[1]) + (parts[2] + parts[3]), axis=0, keepdims=True)
    return total * (1.0 / D)


def _layernorm_coeffs(ref, t, scale):
    m = _row_mean(lambda r: ref[t, 8 * r:8 * r + 8, :])
    v = _row_mean(lambda r: jnp.square(ref[t, 8 * r:8 * r + 8, :] - m))
    a = jax.lax.rsqrt(v + 1e-5) * scale
    return jnp.broadcast_to(a, (16, LANES)), jnp.broadcast_to(m * a, (16, LANES))


def _gate(z):
    out = []
    for i in range(0, z.shape[0], 32):
        g, u = z[i:i + 16], z[i + 16:i + 32]
        out.append(u * jnp.tanh(g) + u)
    return jnp.concatenate(out, 0)


def _pair(p, q):
    low = jax.lax.broadcasted_iota(jnp.int32, p[0].shape, 1) < 64
    return (p[:3] + [jnp.where(low, p[3], p[3] - q[3])],
            q[:3] + [jnp.where(low, q[3], q[4] - p[4])],
            jnp.where(low, q[4], p[4]))


class _Quad:
    def __init__(self, v):
        self.v = list(v)

    def __add__(self, o):
        return _Quad(a + b for a, b in zip(self.v, o.v))

    def __sub__(self, o):
        return _Quad(a - b for a, b in zip(self.v, o.v))


def _quads(b):
    return [_Quad([b[2 * i][2 * j], b[2 * i][2 * j + 1], b[2 * i + 1][2 * j], b[2 * i + 1][2 * j + 1]])
            for i in range(2) for j in range(2)]


def _lhs_combo(n, a11, a12, a21, a22):
    return (lambda: a11 + a22, lambda: a21 + a22, lambda: a11, lambda: a22,
            lambda: a11 + a12, lambda: a21 - a11, lambda: a12 - a22)[n]()


def _rhs_combo(n, b11, b12, b21, b22):
    return (lambda: b11 + b22, lambda: b11, lambda: b12 - b22, lambda: b21 - b11,
            lambda: b22, lambda: b11 + b12, lambda: b21 + b22)[n]()


def _combos2(combo, blocks, emit):
    quads = _quads(blocks)
    for a in range(7):
        outer = combo(a, *quads)
        for b in range(7):
            emit(a, b, combo(b, *outer.v))


_USES = ({0: 1, 3: 1}, {2: 1, 3: -1}, {1: 1, 3: 1}, {0: 1, 2: 1}, {0: -1, 1: 1}, {3: 1}, {0: 1})


def _strassen(mm, fin, order, init=None):
    part = [None] * 4 if init is None else [(1, t) for t in init]
    left = [4, 2, 2, 4]
    for n in order:
        m = mm(n)
        for o, sign in _USES[n].items():
            if part[o] is None:
                part[o] = (sign, m)
            elif part[o][0] < 0:
                part[o] = (1, m - part[o][1])
            else:
                part[o] = (1, part[o][1] + m if sign > 0 else part[o][1] - m)
            left[o] -= 1
            if not left[o]:
                fin(o // 2, o % 2, part[o][1])


def _strassen2(mm, fin, init, o1, o2):
    def outer(a):
        out = [None] * 4

        def keep(i, j, v):
            out[2 * i + j] = v

        _strassen(lambda b: mm(a, b), keep, o2)
        return _Quad(out)

    def fin_quad(i, j, quad):
        for n, v in enumerate(quad.v):
            fin(2 * i + n // 2, 2 * j + n % 2, v)

    _strassen(outer, fin_quad, o1, _quads(init))


def make(ahead=3, prof=False, o1='1475326', o2='3524716', o3='3524716', o4='3524716', hrows=4, prep_mxu=False, flags=None, n_early=3, group=9, layers=2, do_a=True, do_b=True, order="k0 q0 v0 S0 P0 k1 q1 v1 S1 P1 k2 q2 v2 S2 P2 k3 q3 v3 N S3 P3 o0 o1 o2 o3"):
    import contextlib
    scope = jax.named_scope if prof else (lambda name: contextlib.nullcontext())
    ob = lambda t: [int(c) - 1 for c in t]

    def kernel(x_hbm, wqkv_hbm, wo_hbm, wg_hbm, wu_hbm, wd_hbm, o_hbm,
               xio, xs, ys, wqkv_raw, wo_raw, wg_raw, wu_raw, wd_raw,
               tmp, wa, wp, wr, wd, kv, xa, xc, xr, acc, ln, sem_x, sem_a, sem_f, sem_o):
        wa_w, wp_w, wr_w, wd_w, kv_w, xa_w, xc_w, xr_w = [t.bitcast(u32) for t in (wa, wp, wr, wd, kv, xa, xc, xr)]

        def aligned(i, n):
            return i * n if isinstance(i, int) else pl.multiple_of(i * n, n)

        def x_copy(t):
            return pltpu.make_async_copy(x_hbm.at[:, pl.ds(aligned(t, LANES), LANES)], xio.at[t], sem_x.at[t])

        def o_copy(t):
            return pltpu.make_async_copy(xio.at[t], o_hbm.at[:, pl.ds(aligned(t, LANES), LANES)], sem_o.at[t])

        def f_copies(n):
            return [pltpu.make_async_copy(src.at[:, pl.ds(aligned(n, FP), FP)], dst.at[n], sem_f.at[3 * n + i])
                    for i, (src, dst) in enumerate(((wg_hbm, wg_raw), (wu_hbm, wu_raw), (wd_hbm, wd_raw)))]

        def qkv_copy(kt):
            rows = pl.ds(kt * LANES, min(LANES, D - kt * LANES))
            return pltpu.make_async_copy(wqkv_hbm.at[rows], wqkv_raw.at[rows], sem_a.at[kt])

        wo_copy = pltpu.make_async_copy(wo_hbm, wo_raw, sem_a.at[9])

        def store_paired(m, row, p, q):
            p, q, r = _pair(p, q)
            for n, t in enumerate(p + q + [r]):
                wa[m, n, pl.ds(row, 16), :] = t.astype(bf16)

        def prep_wo():
            w32 = wo_raw[...].astype(f32)
            for n in range(5):
                c0 = min(n * LANES, D - LANES)
                tmp[n, 0:D, :] = w32[:, c0:c0 + LANES]
            tiles = []
            for n in range(5):
                rows = jnp.concatenate([tmp[n, pl.ds(hh * HD + d, 16, stride=DH), :]
                                        for hh in range(2) for d in range(DH)], 0).astype(bf16)
                tiles.append([rows[k0:k0 + LANES].T[(64 if n == 4 else 0):] for k0 in KROWS])
            full = [jnp.concatenate([t[k] for t in tiles], 0) for k in range(5)]
            for d in range(HD // 16):
                store_paired(3, 16 * d, [t[16 * d:16 * d + 16].astype(f32) for t in full],
                             [t[HD + 16 * d:HD + 16 * d + 16].astype(f32) for t in full])

        def transpose_qkv(kt, _):
            for c in range(5):
                @pl.when(kt == c)
                def _():
                    qkv_copy(c).wait()
                    if c + ahead < 5:
                        qkv_copy(c + ahead).start()
                    elif c + ahead == 5:
                        for t in range(BT, 2 * BT):
                            x_copy(t).start()
            rows = pl.ds(pl.multiple_of(jnp.minimum(kt * LANES, D - LANES), 64), LANES)
            tmp[kt] = wqkv_raw[rows, :].T.astype(f32)

        def permute_qkv(m, _):
            for d in range(DH):
                p, q = [[tmp[k, pl.ds(m * D + hh * HD + d, 16, stride=DH), :] for k in range(5)] for hh in range(2)]
                store_paired(m, 16 * d, p, q)

        def prep_piece(n):
            eye = (jax.lax.broadcasted_iota(jnp.int32, (LANES, LANES), 0)
                   == jax.lax.broadcasted_iota(jnp.int32, (LANES, LANES), 1)).astype(f32).astype(bf16)

            def transposed(tile):
                if prep_mxu:
                    return jax.lax.dot_general(eye, tile, (((1,), (1,)), ((), ())), preferred_element_type=f32)
                return tile.T.astype(f32)

            for m, raw in enumerate((wg_raw, wu_raw)):
                for c in range(4):
                    row = 32 * c + 16 * m
                    tt = [transposed(raw[n, k0:k0 + LANES, c * LANES:(c + 1) * LANES]) for k0 in KROWS]
                    paired = [_pair([t[16 * i:16 * i + 16] for t in tt], [t[64 + 16 * i:80 + 16 * i] for t in tt])
                              for i in range(4)]
                    for i in range(4):
                        wr[n, 128 * i + row:128 * i + row + 16, :] = paired[i][2].astype(bf16)
                    for s in range(2):
                        def emit(a, b, v):
                            wp[n, s, a, b, row:row + 16, :] = v.astype(bf16)
                        _combos2(_lhs_combo, [t[s] for t in paired], emit)
            for r in range(9):
                blocks = [[wd_raw[n, 144 * i + 16 * r:144 * i + 16 * r + 16, k * LANES:(k + 1) * LANES].astype(f32)
                           for k in range(4)] for i in range(4)]

                def emit(a, b, v):
                    wd[n, a, b, 16 * r:16 * r + 16, :] = v.astype(bf16)
                _combos2(_lhs_combo, blocks, emit)

        def attn_inputs(i):
            for j in range(BT):
                attn_input(j, i * BT + j)

        def attn_input(j, t):
            a, b = _layernorm_coeffs(xs, t, 1.0)
            for r in range(0, D, 16):
                xa[j, r:r + 16, :] = (xs[t, r:r + 16, :] * a - b).astype(bf16)

        def project(m, x, init=None):
            lhs = lambda lo, hi: _half(jnp.concatenate([wa_w[m, n] for n in range(lo, hi)], 1))
            r = _dot(lhs(8, 9), x[448:576])
            rp, rq = (r, r) if init is None else (r + init[:HD], r + init[HD:])
            return (rp + _dot(lhs(0, 4), x[0:512]),
                    rq + _dot(lhs(4, 8), jnp.concatenate([x[0:448], x[512:576]], 0)))

        def attn_block(i):
            t0 = i * BT
            lane8 = jax.lax.broadcasted_iota(jnp.int32, (8, LANES), 1)
            lane16 = jax.lax.broadcasted_iota(jnp.int32, (16, LANES), 1)
            q, prob, o = {}, {}, {}

            def shifts(m, j, r):
                prev, cur = kv_w[m, j, 8 * r:8 * r + 8], kv_w[m, j + 1, 8 * r:8 * r + 8]
                out = [cur] + [pltpu.roll(jnp.where(lane8 >= LANES - DIL * w, prev, cur), DIL * w, 1)
                               for w in range(1, W)]
                return [_half(t).astype(f32) for t in out]

            def scores(j):
                for hh in range(2):
                    logits = None
                    for d in range(DH):
                        qd = q[j][hh][16 * d:16 * d + 16]
                        terms = [qd * t for t in shifts(0, j, hh * DH + d)]
                        logits = terms if d == 0 else [a + b for a, b in zip(logits, terms)]
                    logits = [t * (DH ** -0.5) for t in logits]
                    if j == 0:
                        pos = lane16 + t0 * LANES
                        logits = logits[:1] + [jnp.where(pos >= DIL * w, logits[w], -1e9) for w in range(1, W)]
                    mx = functools.reduce(jnp.maximum, logits)
                    e = [jnp.exp(t - mx) for t in logits]
                    inv = 1.0 / functools.reduce(jnp.add, e)
                    prob[j, hh] = [t * inv for t in e]

            def values(j):
                rows = []
                for hh in range(2):
                    for d in range(DH):
                        terms = [a * b for a, b in zip(prob[j, hh], shifts(1, j, hh * DH + d))]
                        rows.append(functools.reduce(jnp.add, terms))
                o[j] = jnp.concatenate(rows, 0).astype(bf16)

            for step in order.split():
                op, js = step[0], [int(c) for c in step[1:]]
                if op == "S":
                    scores(js[0])
                elif op == "P":
                    values(js[0])
                elif op == "N":
                    attn_inputs(jnp.minimum(i + 1, NB - 1))
                else:
                    m = "qkvo".index(op)
                    src = [o[j] if op == "o" else _half(xa_w[j]) for j in js]
                    init = jnp.concatenate([xs[t0 + j] for j in js], 1) if op == "o" else None
                    halves = project(m, jnp.concatenate(src, 1), init)
                    for n, j in enumerate(js):
                        part = [t[:, n * LANES:(n + 1) * LANES] for t in halves]
                        if op == "q":
                            q[j] = part
                        for hh in range(2):
                            rows = slice(hh * HD, (hh + 1) * HD)
                            if op == "o":
                                ys[t0 + j, rows, :] = part[hh]
                            elif op != "q":
                                kv[m - 1, j + 1, rows, :] = part[hh].astype(bf16)
            for m in range(2):
                kv_w[m, 0] = kv_w[m, BT]

        def ffn_inputs(i):
            coeffs = [(ln[j, 0], ln[j, 1]) for j in range(BT)]
            for r in (4, 8, 5, 9, 6, 10, 7, 11, 0, 1, 2, 3):
                lo = 16 * (r if r < 8 else r - 4)
                blocks = [[ys[i * BT + j, k0:k0 + 16, :] * coeffs[j][0] - coeffs[j][1] for j in range(BT)]
                          for k0 in (lo, 128 + lo, 256 + lo, 384 + 16 * r)]
                if r >= 4:
                    for j in range(BT):
                        xr[j, 16 * r - 64:16 * r - 48, :] = blocks[3][j].astype(bf16)

                def emit(a, b, v):
                    xc[a, b, 16 * r:16 * r + 16, :] = v.astype(bf16)
                _combos2(_rhs_combo, blocks, emit)

        def ffn_stats(j, t):
            ln[j, 0], ln[j, 1] = _layernorm_coeffs(ys, t, 0.5)

        def ffn_block(i):
            t0 = i * BT
            hc = []
            ffn_inputs(i)
            shared = lambda n: _dot(_half(wr_w[n]), _half(jnp.concatenate([xr_w[j] for j in range(BT)], 1)))
            early = [shared(n) for n in range(n_early)]
            for n in range(NP):
                r = early[n] if n < n_early else shared(n)
                if n in (3, 4, 5, 6):
                    ffn_stats(n - 3, jnp.minimum(i + 1, NB - 1) * BT + n - 3)
                init = [[r[i * 128:(i + 1) * 128, j * LANES:(j + 1) * LANES] for j in range(4)] for i in range(4)]
                for s in range(2):
                    h = [[None] * 4 for _ in range(4)]

                    def mm(a, b):
                        rhs = jnp.concatenate([xc_w[a, b, 0:32], xc_w[a, b, 32 + 32 * s:64 + 32 * s]], 0)
                        return _dot(_half(wp_w[n, s, a, b]), _half(rhs))

                    def fin(i, j, v):
                        h[i][j] = _gate(v)
                    _strassen2(mm, fin, init, ob(o1), ob(o2))
                    for i0 in range(0, 4, hrows):
                        combos = {}

                        def emit(a, b, v):
                            combos[a, b] = v.astype(bf16)
                        _combos2(_rhs_combo, [[jnp.concatenate([h[i][j][16 * c:16 * c + 16] for i in range(i0, i0 + hrows)], 0)
                                               for j in range(4)] for c in range(4)], emit)
                        hc.append(combos)
                if (n + 1) % group == 0:
                    def down(a, b):
                        lhs = jnp.concatenate([wd_w[m, a, b] for m in range(n + 1 - group, n + 1)], 1)
                        t = _dot(_half(lhs), jnp.concatenate([c[a, b] for c in hc], 0))
                        return t if n < group else acc[a, b] + t
                    if n < NP - 1:
                        for a in (1, 4, 2, 3, 5, 6, 0):
                            for b in range(7):
                                acc[a, b] = down(a, b)
                    else:
                        def out(i, j, v):
                            xs[t0 + j, 144 * i:144 * (i + 1), :] = v
                            xio[t0 + j, 144 * i:144 * (i + 1), :] = v.astype(bf16)
                        _strassen2(down, out, [[ys[t0 + j, 144 * i:144 * (i + 1), :] for j in range(4)] for i in range(4)], ob(o3), ob(o4))
                    hc = []

        def load_x(t, _):
            x_copy(t).wait()
            xs[t] = xio[t].astype(f32)

        wo_copy.start()
        for t in range(BT):
            x_copy(t).start()
        with scope('wo_wait'):
            wo_copy.wait()
        for c in range(ahead):
            qkv_copy(c).start()
        with scope('prep_wo'):
            prep_wo()
        with scope('load_x'):
            jax.lax.fori_loop(0, BT, load_x, None)

        def layer(l, _):
            for m in range(2):
                kv_w[m, 0] = jnp.zeros((HD, LANES), u32)
            with scope('first_in'):
                attn_inputs(0)

            @pl.when(l == 0)
            def _():
                with scope('tr_qkv'):
                    jax.lax.fori_loop(0, 5, transpose_qkv, None)
                with scope('perm_qkv'):
                    jax.lax.fori_loop(0, 3, permute_qkv, None)

            def attn_step(i, _):
                @pl.when((l == 0) & (i + 1 < NB))
                def _():
                    def next_x(t, _):
                        load_x(t, None)
                        pl.when(t + BT < NT)(lambda: x_copy(t + BT).start())

                    def start_piece(n, _):
                        for cp in f_copies(n):
                            cp.start()
                    jax.lax.fori_loop((i + 1) * BT, (i + 2) * BT, next_x, None)
                    jax.lax.fori_loop(3 * i, 3 * i + 3, start_piece, None)

                with scope('attn_blk'):
                    attn_block(i)

            jax.lax.fori_loop(0, NB, attn_step, None)

            @pl.when(l == 0)
            def _():
                def step(n, _):
                    for cp in f_copies(n):
                        cp.wait()
                    prep_piece(n)
                with scope('prep'):
                    jax.lax.fori_loop(0, NP, step, None)

            def ffn_step(i, _):
                if do_b:
                    ffn_block(i)
                else:
                    xs[i] = ys[i]
                    xio[i] = ys[i].astype(bf16)

                @pl.when(l == layers - 1)
                def _():
                    for j in range(BT):
                        o_copy(i * BT + j).start()

            with scope('stats'):
                [ffn_stats(j, j) for j in range(BT)]
            with scope('ffn'):
                jax.lax.fori_loop(0, NB, ffn_step, None)

        jax.lax.fori_loop(0, layers, layer, None)
        for t in range(NT):
            o_copy(t).wait()

    @jax.jit
    def f(A_x, A_wqkv, A_wo, B_x, B_w_gate, B_w_up, B_w_down):
        del B_x
        hbm = pl.BlockSpec(memory_space=pltpu.HBM)
        out = pl.pallas_call(
            kernel,
            out_shape=jax.ShapeDtypeStruct((D, S), bf16),
            in_specs=[hbm] * 6,
            out_specs=hbm,
            scratch_shapes=[
                pltpu.VMEM((NT, D, LANES), bf16),
                pltpu.VMEM((NT, D, LANES), f32),
                pltpu.VMEM((NT, D, LANES), f32),
                pltpu.VMEM((D, 3 * D), bf16),
                pltpu.VMEM((D, D), bf16),
                pltpu.VMEM((NP, D, FP), bf16),
                pltpu.VMEM((NP, D, FP), bf16),
                pltpu.VMEM((NP, D, FP), bf16),
                pltpu.VMEM((5, 3 * D, LANES), f32),
                pltpu.VMEM((4, 9, HD, LANES), bf16),
                pltpu.VMEM((NP, 2, 7, 7, 128, LANES), bf16),
                pltpu.VMEM((NP, 512, LANES), bf16),
                pltpu.VMEM((NP, 7, 7, 144, LANES), bf16),
                pltpu.VMEM((2, BT + 1, D, LANES), bf16),
                pltpu.VMEM((BT, D, LANES), bf16),
                pltpu.VMEM((7, 7, 192, LANES), bf16),
                pltpu.VMEM((BT, 128, LANES), bf16),
                pltpu.VMEM((7, 7, 144, LANES), f32),
                pltpu.VMEM((BT, 2, 16, LANES), f32),
                pltpu.SemaphoreType.DMA((NT,)),
                pltpu.SemaphoreType.DMA((10,)),
                pltpu.SemaphoreType.DMA((3 * NP,)),
                pltpu.SemaphoreType.DMA((NT,)),
            ],
            compiler_params=pltpu.CompilerParams(vmem_limit_bytes=120 * 2**20, flags=flags),
        )(A_x[0].T, A_wqkv, A_wo, B_w_gate, B_w_up, B_w_down.T)
        return out.T[None]

    return f


pallas_interleave_layers__sliding_local_dilated__glu_gated_glu__prompt_kernel = make()
```

```python
import functools

import jax
import jax.numpy as jnp
import jax.experimental.pallas as pl
import jax.experimental.pallas.tpu as pltpu

S, D, F = 2048, 576, 4608
DH, W, DIL = 18, 8, 2
LANES = 128
HD = D // 2
QD = D // 4
NT = S // LANES
BT = 4
NB = NT // BT
FP = 512
NP = F // FP
KROWS = (0, 128, 256, 384, 448)
f32, bf16 = jnp.float32, jnp.bfloat16


def _dot(a, b):
    return jnp.dot(a, b, preferred_element_type=f32)


def _load(ref, *idx, rows=None):
    if rows is not None:
        idx += (slice(rows[0] // 2, rows[1] // 2),)
    return pltpu.bitcast(ref.bitcast(jnp.uint32)[idx], bf16)


def _row_mean(rows):
    parts = [rows(0), rows(16)]
    for n, r in enumerate(range(32, D, 16)):
        parts[n % 2] = parts[n % 2] + rows(r)
    return jnp.sum(parts[0] + parts[1], axis=0, keepdims=True) * (1.0 / D)


def _layernorm_coeffs(rows, scale):
    m = _row_mean(rows)
    v = _row_mean(lambda r: jnp.square(rows(r) - m))
    a = jax.lax.rsqrt(v + 1e-5) * scale
    return jnp.broadcast_to(a, (16, LANES)), jnp.broadcast_to(m * a, (16, LANES))


def _pair(p, q):
    low = jax.lax.broadcasted_iota(jnp.int32, p[0].shape, 1) < 64
    return (p[:3] + [jnp.where(low, p[3], p[3] - q[3])],
            q[:3] + [jnp.where(low, q[3], q[4] - p[4])],
            jnp.where(low, q[4], p[4]))


class _Quad:
    def __init__(self, v):
        self.v = list(v)

    def __add__(self, o):
        return _Quad(a + b for a, b in zip(self.v, o.v))

    def __sub__(self, o):
        return _Quad(a - b for a, b in zip(self.v, o.v))


def _quads(b):
    return [_Quad(b[2 * i + n // 2][2 * j + n % 2] for n in range(4)) for i in range(2) for j in range(2)]


def _lhs_terms(a11, a12, a21, a22):
    return [a11 + a22, a21 + a22, a11, a22, a11 + a12, a21 - a11, a12 - a22]


def _rhs_terms(b11, b12, b21, b22):
    return [b11 + b22, b11, b12 - b22, b21 - b11, b22, b11 + b12, b21 + b22]


def _operands(terms, blocks):
    return [terms(*outer.v) for outer in terms(*_quads(blocks))]


_USES = ({0: 1, 3: 1}, {2: 1, 3: -1}, {1: 1, 3: 1}, {0: 1, 2: 1}, {0: -1, 1: 1}, {3: 1}, {0: 1})
_UP_ORDER = ((0, 3, 6, 4, 2, 1, 5), (1, 3, 0, 6, 5, 2, 4))
_DOWN_ORDER = ((1, 3, 4, 6, 0, 2, 5), (2, 4, 1, 3, 6, 0, 5))


def _collect(product, order, init=()):
    part = {o: (1, t) for o, t in enumerate(init)}
    for n in order:
        m = product(n)
        for o, sign in _USES[n].items():
            if o not in part:
                part[o] = (sign, m)
            elif part[o][0] < 0:
                part[o] = (1, m - part[o][1])
            else:
                part[o] = (1, part[o][1] + m if sign > 0 else part[o][1] - m)
    return [part[o][1] for o in range(4)]


def _strassen(product, init, order):
    z = _collect(lambda a: _Quad(_collect(lambda b: product(a, b), order[1])), order[0], _quads(init))
    return [[z[2 * (i // 2) + j // 2].v[2 * (i % 2) + j % 2] for j in range(4)] for i in range(4)]


def _kernel(x_hbm, wqkv_hbm, wo_hbm, wg_hbm, wu_hbm, wd_hbm, o_hbm,
            xs, ys, wqkv_raw, wo_raw, wg_raw, wu_raw, wd_raw,
            tmp, wa, wp, wr, wd, kv, xa, ln, sem_x, sem_a, sem_f, sem_o):
    kv_words = kv.bitcast(jnp.uint32)

    def block(i, n):
        return pl.ds(i * n if isinstance(i, int) else pl.multiple_of(i * n, n), n)

    def x_copy(t):
        return pltpu.make_async_copy(x_hbm.at[:, block(t, LANES)], xs.at[t], sem_x.at[t])

    def o_copy(t):
        return pltpu.make_async_copy(xs.at[t], o_hbm.at[:, block(t, LANES)], sem_o.at[t])

    def glu_copies(n):
        return [pltpu.make_async_copy(src.at[:, block(n, FP)], dst.at[n], sem_f.at[3 * n + i])
                for i, (src, dst) in enumerate(((wg_hbm, wg_raw), (wu_hbm, wu_raw), (wd_hbm, wd_raw)))]

    def qkv_copy(k):
        rows = pl.ds(k * LANES, min(LANES, D - k * LANES))
        return pltpu.make_async_copy(wqkv_hbm.at[rows], wqkv_raw.at[rows], sem_a.at[k])

    wo_copy = pltpu.make_async_copy(wo_hbm, wo_raw, sem_a.at[5])
    waves = [[qkv_copy(k)] for k in range(5)] + [
        [wo_copy],
        [x_copy(t) for t in range(BT)],
        [x_copy(t) for t in range(BT, 2 * BT)],
        [x_copy(t) for t in range(2 * BT, NT)] + glu_copies(0) + glu_copies(1),
        [cp for n in range(2, NP) for cp in glu_copies(n)],
    ]

    def start_wave(n):
        for cp in waves[n]:
            cp.start()

    def store_paired(m, row, p, q):
        p, q, r = _pair(p, q)
        for n, t in enumerate(p + q + [r]):
            wa[m, n, row:row + 16, :] = t.astype(bf16)

    def transpose_qkv(k, _):
        for c in range(5):
            @pl.when(k == c)
            def _():
                qkv_copy(c).wait()
                start_wave(c + 3)
        rows = pl.ds(pl.multiple_of(jnp.minimum(k * LANES, D - LANES), 64), LANES)
        tmp[k, 0:3 * D, :] = wqkv_raw[rows, :].T.astype(f32)

    def reorder_qkv(m, _):
        for d in range(DH):
            p, q = [[tmp[k, pl.ds(m * D + hh * HD + d, 16, stride=DH), :] for k in range(5)] for hh in range(2)]
            store_paired(m, 16 * d, p, q)

    def prepare_wo():
        w32 = wo_raw[...].astype(f32)
        tiles = []
        for n, c0 in enumerate(KROWS):
            tmp[n, 0:D, :] = w32[:, c0:c0 + LANES]
            rows = jnp.concatenate([tmp[n, pl.ds(hh * HD + d, 16, stride=DH), :]
                                    for hh in range(2) for d in range(DH)], 0).astype(bf16)
            tiles.append([rows[k0:k0 + LANES].T[n * LANES - c0:] for k0 in KROWS])
        full = [jnp.concatenate([t[k] for t in tiles], 0) for k in range(5)]
        for r in range(0, HD, 16):
            store_paired(3, r, [t[r:r + 16].astype(f32) for t in full],
                         [t[HD + r:HD + r + 16].astype(f32) for t in full])

    def prepare_glu(n, _):
        for cp in glu_copies(n):
            cp.wait()
        for m, raw in enumerate((wg_raw, wu_raw)):
            for c in range(4):
                row = 32 * c + 16 * m
                tt = {k: raw[n, KROWS[k]:KROWS[k] + LANES, c * LANES:(c + 1) * LANES].T.astype(f32)
                      for k in (3, 4, 0, 1, 2)}
                paired = [_pair([tt[k][16 * i:16 * i + 16] for k in range(5)],
                                [tt[k][64 + 16 * i:80 + 16 * i] for k in range(5)]) for i in range(4)]
                for i in range(4):
                    wr[n, 128 * i + row:128 * i + row + 16, :] = paired[i][2].astype(bf16)
                for s in range(2):
                    for a, terms in enumerate(_operands(_lhs_terms, [t[s] for t in paired])):
                        for b, v in enumerate(terms):
                            wp[n, s, a, b, row:row + 16, :] = v.astype(bf16)
        for r in range(0, QD, 16):
            blocks = [[wd_raw[n, QD * i + r:QD * i + r + 16, c * LANES:(c + 1) * LANES].astype(f32)
                       for c in range(4)] for i in range(4)]
            for a, terms in enumerate(_operands(_lhs_terms, blocks)):
                for b, v in enumerate(terms):
                    wd[n, a, b, r:r + 16, :] = v.astype(bf16)

    def attn_inputs(i):
        for j in range(BT):
            def rows(r):
                return _load(xs, i * BT + j, rows=(r, r + 16)).astype(f32)
            a, b = _layernorm_coeffs(rows, 1.0)
            for r in range(0, D, 16):
                xa[j, r:r + 16, :] = (rows(r) * a - b).astype(bf16)

    def project(names, steps, x):
        parts = {"P": (range(0, 4), x[0:512]),
                 "Q": (range(4, 8), jnp.concatenate([x[0:448], x[512:576]], 0)),
                 "R": (range(8, 9), x[448:576])}
        z = {}
        for step in steps.split():
            tiles, rhs = parts[step[1]]
            z[step] = _dot(jnp.concatenate([_load(wa, "qkvo".index(step[0]), n) for n in tiles], 1), rhs)
        return [jnp.concatenate([z[c + "R"] + z[c + "P"], z[c + "R"] + z[c + "Q"]], 0) for c in names]

    def attn_block(i):
        lane = jax.lax.broadcasted_iota(jnp.int32, (8, LANES), 1)

        def window(m, j, r):
            prev, cur = kv_words[m, j, 8 * r:8 * r + 8], kv_words[m, j + 1, 8 * r:8 * r + 8]
            out = [cur] + [pltpu.roll(jnp.where(lane >= LANES - DIL * w, prev, cur), DIL * w, 1)
                           for w in range(1, W)]
            return [pltpu.bitcast(t, bf16).astype(f32) for t in out]

        heads = []
        for j in range(BT):
            q, k, v = project("qkv", "kR qR vR kP qP kQ qQ vP vQ", _load(xa, j))
            kv[0, j + 1] = k.astype(bf16)
            kv[1, j + 1] = v.astype(bf16)
            if j == 0:
                kv_words[1, 0] = jnp.where(i == 0, kv_words[1, 1][:, 0:1], kv_words[1, 0])
            prob = []
            for hh in range(2):
                for d in range(DH):
                    r = hh * DH + d
                    terms = [q[16 * r:16 * r + 16] * t for t in window(0, j, r)]
                    logits = terms if d == 0 else [a + b for a, b in zip(logits, terms)]
                logits = [t * (DH ** -0.5) for t in logits]
                if j == 0:
                    pos = jax.lax.broadcasted_iota(jnp.int32, (16, LANES), 1) + i * (BT * LANES)
                    logits = [jnp.where(pos >= DIL * w, t, -1e9) for w, t in enumerate(logits)]
                top = functools.reduce(jnp.maximum, logits)
                e = [jnp.exp(t - top) for t in logits]
                inv = 1.0 / functools.reduce(jnp.add, e)
                prob.append([t * inv for t in e])
            rows = [functools.reduce(jnp.add, [a * b for a, b in zip(prob[r // DH], window(1, j, r))])
                    for r in range(2 * DH)]
            heads.append(jnp.concatenate(rows, 0).astype(bf16))
        for m in range(2):
            kv_words[m, 0] = kv_words[m, BT]
        attn_inputs(jnp.minimum(i + 1, NB - 1))
        for j in range(BT):
            x = _load(xs, i * BT + j).astype(f32)
            ys[i * BT + j] = project("o", "oR oP oQ", heads[j])[0] + x

    def glu_coeffs(i):
        for j in range(BT):
            ln[j, 0], ln[j, 1] = _layernorm_coeffs(lambda r: ys[i * BT + j, r:r + 16, :], 0.5)

    def gated(z, c):
        g, u = z[32 * c:32 * c + 16], z[32 * c + 16:32 * c + 32]
        return u * jnp.tanh(g) + u

    def glu_block(i, last):
        t0 = i * BT
        x = {r: [ys[t0 + j, r:r + 16, :] * ln[j, 0] - ln[j, 1] for j in range(BT)] for r in range(0, D, 16)}
        glu_coeffs(jnp.minimum(i + 1, NB - 1))
        x_ops = [_operands(_rhs_terms, [x[r], x[128 + r], x[256 + r], x[k3 + r]])
                 for k3, lo in ((384, 0), (448, 64)) for r in range(lo, 128, 16)]
        x_ops = [[jnp.concatenate([t[a][b] for t in x_ops], 0).astype(bf16) for b in range(7)] for a in range(7)]
        x_tail = jnp.concatenate([jnp.concatenate(x[r], 1) for r in range(448, D, 16)], 0).astype(bf16)
        early = [_dot(_load(wr, n), x_tail) for n in range(2)]
        h_ops = []
        for n in range(NP):
            shared = early[n] if n < len(early) else _dot(_load(wr, n), x_tail)
            init = [[shared[128 * b:128 * b + 128, LANES * j:LANES * j + LANES] for j in range(4)] for b in range(4)]
            for s in range(2):
                def up(a, b):
                    t = x_ops[a][b]
                    return _dot(_load(wp, n, s, a, b), jnp.concatenate([t[0:64], t[64 + 64 * s:128 + 64 * s]], 0))
                z = _strassen(up, init, _UP_ORDER)
                h = [[jnp.concatenate([gated(t[j], c) for t in z], 0) for j in range(4)] for c in range(4)]
                h_ops.append([[v.astype(bf16) for v in terms] for terms in _operands(_rhs_terms, h)])

        def down(a, b):
            return _dot(jnp.concatenate([_load(wd, n, a, b) for n in range(NP)], 1),
                        jnp.concatenate([t[a][b] for t in h_ops], 0))
        init = [[ys[t0 + j, QD * b:QD * b + QD, :] for j in range(4)] for b in range(4)]
        out = _strassen(down, init, _DOWN_ORDER)
        for j in range(BT):
            for b in ((2, 3, 0, 1) if j < 2 else (0, 1, 2, 3)):
                xs[t0 + j, QD * b:QD * b + QD, :] = out[b][j].astype(bf16)
            if j % 2:
                @pl.when(last)
                def _():
                    o_copy(t0 + j - 1).start()
                    o_copy(t0 + j).start()

    for n in range(3):
        start_wave(n)
    jax.lax.fori_loop(0, 5, transpose_qkv, None)
    jax.lax.fori_loop(0, 3, reorder_qkv, None)
    wo_copy.wait()
    prepare_wo()
    for t in range(BT):
        x_copy(t).wait()

    def layer(l, _):
        for m in range(2):
            kv[m, 0] = jnp.zeros((D, LANES), bf16)
        attn_inputs(0)

        def attn_step(i, _):
            for step, (lo, hi) in enumerate(((BT, 2 * BT), (2 * BT, NT))):
                @pl.when((l == 0) & (i == step))
                def _():
                    jax.lax.fori_loop(lo, hi, lambda t, _: x_copy(t).wait(), None)
                    start_wave(8 + step)
            attn_block(i)

        jax.lax.fori_loop(0, NB, attn_step, None)
        pl.when(l == 0)(lambda: jax.lax.fori_loop(0, NP, prepare_glu, None))
        glu_coeffs(0)
        jax.lax.fori_loop(0, NB, lambda i, _: glu_block(i, l == 1), None)

    jax.lax.fori_loop(0, 2, layer, None)
    for t in range(NT):
        o_copy(t).wait()


@jax.jit
def pallas_interleave_layers__sliding_local_dilated__glu_gated_glu__prompt_kernel(
    A_x: jax.Array,
    A_wqkv: jax.Array,
    A_wo: jax.Array,
    B_x: jax.Array,
    B_w_gate: jax.Array,
    B_w_up: jax.Array,
    B_w_down: jax.Array,
):
    del B_x
    hbm = pl.BlockSpec(memory_space=pltpu.HBM)
    out = pl.pallas_call(
        _kernel,
        out_shape=jax.ShapeDtypeStruct((D, S), bf16),
        in_specs=[hbm] * 6,
        out_specs=hbm,
        scratch_shapes=[
            pltpu.VMEM((NT, D, LANES), bf16),
            pltpu.VMEM((NT, D, LANES), f32),
            pltpu.VMEM((D, 3 * D), bf16),
            pltpu.VMEM((D, D), bf16),
            pltpu.VMEM((NP, D, FP), bf16),
            pltpu.VMEM((NP, D, FP), bf16),
            pltpu.VMEM((NP, D, FP), bf16),
            pltpu.VMEM((5, 3 * D + 24, LANES), f32),
            pltpu.VMEM((4, 9, HD, LANES), bf16),
            pltpu.VMEM((NP, 2, 7, 7, 128, LANES), bf16),
            pltpu.VMEM((NP, 512, LANES), bf16),
            pltpu.VMEM((NP, 7, 7, QD, LANES), bf16),
            pltpu.VMEM((2, BT + 1, D, LANES), bf16),
            pltpu.VMEM((BT, D, LANES), bf16),
            pltpu.VMEM((BT, 2, 16, LANES), f32),
            pltpu.SemaphoreType.DMA((NT,)),
            pltpu.SemaphoreType.DMA((6,)),
            pltpu.SemaphoreType.DMA((3 * NP,)),
            pltpu.SemaphoreType.DMA((NT,)),
        ],
        compiler_params=pltpu.CompilerParams(vmem_limit_bytes=120 * 2**20),
    )(A_x.reshape(S, D).T, A_wqkv, A_wo, B_w_gate, B_w_up, B_w_down.T)
    return out.T.reshape(1, S, D)
```

```python
import functools

import jax
import jax.numpy as jnp
import jax.experimental.pallas as pl
import jax.experimental.pallas.tpu as pltpu

S, D, F = 2048, 576, 4608
DH, W, DIL = 18, 8, 2
LANES = 128
HD = D // 2
QD = D // 4
NT = S // LANES
BT = 4
NB = NT // BT
FP = 512
NP = F // FP
KROWS = (0, 128, 256, 384, 448)
f32, bf16 = jnp.float32, jnp.bfloat16


def _dot(a, b):
    return jnp.dot(a, b, preferred_element_type=f32)


def _load(ref, *idx):
    return pltpu.bitcast(ref.bitcast(jnp.uint32)[idx], bf16)


def _row_mean(rows):
    parts = [rows(0), rows(16)]
    for n, r in enumerate(range(32, D, 16)):
        parts[n % 2] = parts[n % 2] + rows(r)
    return jnp.sum(parts[0] + parts[1], axis=0, keepdims=True) * (1.0 / D)


def _layernorm_coeffs(rows, scale):
    m = _row_mean(rows)
    v = _row_mean(lambda r: jnp.square(rows(r) - m))
    a = jax.lax.rsqrt(v + 1e-5) * scale
    return jnp.broadcast_to(a, (16, LANES)), jnp.broadcast_to(m * a, (16, LANES))


def _pair(p, q):
    low = jax.lax.broadcasted_iota(jnp.int32, p[0].shape, 1) < 64
    return (p[:3] + [jnp.where(low, p[3], p[3] - q[3])],
            q[:3] + [jnp.where(low, q[3], q[4] - p[4])],
            jnp.where(low, q[4], p[4]))


class _Quad:
    def __init__(self, v):
        self.v = list(v)

    def __add__(self, o):
        return _Quad(a + b for a, b in zip(self.v, o.v))

    def __sub__(self, o):
        return _Quad(a - b for a, b in zip(self.v, o.v))


def _quads(b):
    return [_Quad(b[2 * i + n // 2][2 * j + n % 2] for n in range(4)) for i in range(2) for j in range(2)]


def _lhs_terms(a11, a12, a21, a22):
    return [a11 + a22, a21 + a22, a11, a22, a11 + a12, a21 - a11, a12 - a22]


def _rhs_terms(b11, b12, b21, b22):
    return [b11 + b22, b11, b12 - b22, b21 - b11, b22, b11 + b12, b21 + b22]


def _operands(terms, blocks):
    return [terms(*outer.v) for outer in terms(*_quads(blocks))]


_USES = ({0: 1, 3: 1}, {2: 1, 3: -1}, {1: 1, 3: 1}, {0: 1, 2: 1}, {0: -1, 1: 1}, {3: 1}, {0: 1})
_UP_ORDER = ((0, 3, 6, 4, 2, 1, 5), (1, 3, 0, 6, 5, 2, 4))
_QKV_ORDER = "kR qR vR kP qP kQ qQ vP vQ"
_DOWN_ORDER = ((1, 3, 4, 6, 0, 2, 5), (2, 4, 1, 3, 6, 0, 5))


def _collect(product, order, init=()):
    part = {o: (1, t) for o, t in enumerate(init)}
    for n in order:
        m = product(n)
        for o, sign in _USES[n].items():
            if o not in part:
                part[o] = (sign, m)
            elif part[o][0] < 0:
                part[o] = (1, m - part[o][1])
            else:
                part[o] = (1, part[o][1] + m if sign > 0 else part[o][1] - m)
    return [part[o][1] for o in range(4)]


def _strassen(product, init, order):
    z = _collect(lambda a: _Quad(_collect(lambda b: product(a, b), order[1])), order[0], _quads(init))
    return [[z[2 * (i // 2) + j // 2].v[2 * (i % 2) + j % 2] for j in range(4)] for i in range(4)]


def _kernel(x_hbm, wqkv_hbm, wo_hbm, wg_hbm, wu_hbm, wd_hbm, o_hbm,
            xs, ys, wqkv_raw, wo_raw, wg_raw, wu_raw, wd_raw,
            tmp, wa, wp, wr, wd, kv, xa, ln, sem_x, sem_a, sem_f, sem_o):
    kv_words = kv.bitcast(jnp.uint32)

    def block(i, n):
        return pl.ds(i * n if isinstance(i, int) else pl.multiple_of(i * n, n), n)

    def x_copy(t):
        return pltpu.make_async_copy(x_hbm.at[:, block(t, LANES)], xs.at[t], sem_x.at[t])

    def o_copy(t):
        return pltpu.make_async_copy(xs.at[t], o_hbm.at[:, block(t, LANES)], sem_o.at[t])

    def glu_copies(n):
        return [pltpu.make_async_copy(src.at[:, block(n, FP)], dst.at[n], sem_f.at[3 * n + i])
                for i, (src, dst) in enumerate(((wg_hbm, wg_raw), (wu_hbm, wu_raw), (wd_hbm, wd_raw)))]

    def qkv_copy(k):
        rows = pl.ds(k * LANES, min(LANES, D - k * LANES))
        return pltpu.make_async_copy(wqkv_hbm.at[rows], wqkv_raw.at[rows], sem_a.at[k])

    wo_copy = pltpu.make_async_copy(wo_hbm, wo_raw, sem_a.at[5])
    waves = [[qkv_copy(k)] for k in range(5)] + [
        [wo_copy],
        [x_copy(t) for t in range(BT)],
        [x_copy(t) for t in range(BT, 2 * BT)],
        [x_copy(t) for t in range(2 * BT, NT)] + glu_copies(0) + glu_copies(1),
        [cp for n in range(2, NP) for cp in glu_copies(n)],
    ]

    def start_wave(n):
        for cp in waves[n]:
            cp.start()

    def store_paired(m, row, p, q):
        p, q, r = _pair(p, q)
        for n, t in enumerate(p + q + [r]):
            wa[m, n, row:row + 16, :] = t.astype(bf16)

    def transpose_qkv(k, _):
        for c in range(5):
            @pl.when(k == c)
            def _():
                qkv_copy(c).wait()
                start_wave(c + 3)
        rows = pl.ds(pl.multiple_of(jnp.minimum(k * LANES, D - LANES), 64), LANES)
        tmp[k, 0:3 * D, :] = wqkv_raw[rows, :].T.astype(f32)

    def reorder_qkv(m, _):
        for d in range(DH):
            p, q = [[tmp[k, pl.ds(m * D + hh * HD + d, 16, stride=DH), :] for k in range(5)] for hh in range(2)]
            store_paired(m, 16 * d, p, q)

    def prepare_wo():
        w32 = wo_raw[...].astype(f32)
        tiles = []
        for n, c0 in enumerate(KROWS):
            tmp[n, 0:D, :] = w32[:, c0:c0 + LANES]
            rows = jnp.concatenate([tmp[n, pl.ds(hh * HD + d, 16, stride=DH), :]
                                    for hh in range(2) for d in range(DH)], 0).astype(bf16)
            tiles.append([rows[k0:k0 + LANES].T[n * LANES - c0:] for k0 in KROWS])
        full = [jnp.concatenate([t[k] for t in tiles], 0) for k in range(5)]
        for r in range(0, HD, 16):
            store_paired(3, r, [t[r:r + 16].astype(f32) for t in full],
                         [t[HD + r:HD + r + 16].astype(f32) for t in full])

    def prepare_glu(n, _):
        for cp in glu_copies(n):
            cp.wait()
        for m, raw in enumerate((wg_raw, wu_raw)):
            for c in range(4):
                row = 32 * c + 16 * m
                tt = {k: raw[n, KROWS[k]:KROWS[k] + LANES, c * LANES:(c + 1) * LANES].T.astype(f32)
                      for k in (3, 4, 0, 1, 2)}
                paired = [_pair([tt[k][16 * i:16 * i + 16] for k in range(5)],
                                [tt[k][64 + 16 * i:80 + 16 * i] for k in range(5)]) for i in range(4)]
                for i in range(4):
                    wr[n, 128 * i + row:128 * i + row + 16, :] = paired[i][2].astype(bf16)
                for s in range(2):
                    for a, terms in enumerate(_operands(_lhs_terms, [t[s] for t in paired])):
                        for b, v in enumerate(terms):
                            wp[n, s, a, b, row:row + 16, :] = v.astype(bf16)
        for r in range(0, QD, 16):
            blocks = [[wd_raw[n, QD * i + r:QD * i + r + 16, c * LANES:(c + 1) * LANES].astype(f32)
                       for c in range(4)] for i in range(4)]
            for a, terms in enumerate(_operands(_lhs_terms, blocks)):
                for b, v in enumerate(terms):
                    wd[n, a, b, r:r + 16, :] = v.astype(bf16)

    def attn_inputs(i):
        for j in range(BT):
            def rows(r):
                return xs[i * BT + j, r:r + 16, :].astype(f32)
            a, b = _layernorm_coeffs(rows, 1.0)
            for r in range(0, D, 16):
                xa[j, r:r + 16, :] = (rows(r) * a - b).astype(bf16)

    def project(names, steps, x):
        parts = {"P": (range(0, 4), x[0:512]),
                 "Q": (range(4, 8), jnp.concatenate([x[0:448], x[512:576]], 0)),
                 "R": (range(8, 9), x[448:576])}
        z = {}
        for step in steps.split():
            tiles, rhs = parts[step[1]]
            z[step] = _dot(jnp.concatenate([_load(wa, "qkvo".index(step[0]), n) for n in tiles], 1), rhs)
        return [jnp.concatenate([z[c + "R"] + z[c + "P"], z[c + "R"] + z[c + "Q"]], 0) for c in names]

    def attn_block(i):
        lane = jax.lax.broadcasted_iota(jnp.int32, (8, LANES), 1)

        def window(m, j, r):
            prev, cur = kv_words[m, j, 8 * r:8 * r + 8], kv_words[m, j + 1, 8 * r:8 * r + 8]
            out = [cur] + [pltpu.roll(jnp.where(lane >= LANES - DIL * w, prev, cur), DIL * w, 1)
                           for w in range(1, W)]
            return [pltpu.bitcast(t, bf16).astype(f32) for t in out]

        heads = []
        for j in range(BT):
            q, k, v = project("qkv", _QKV_ORDER, _load(xa, j))
            kv[0, j + 1] = k.astype(bf16)
            kv[1, j + 1] = v.astype(bf16)
            if j == 0:
                kv_words[1, 0] = jnp.where(i == 0, kv_words[1, 1][:, 0:1], kv_words[1, 0])
            prob = []
            for hh in range(2):
                for d in range(DH):
                    r = hh * DH + d
                    terms = [q[16 * r:16 * r + 16] * t for t in window(0, j, r)]
                    logits = terms if d == 0 else [a + b for a, b in zip(logits, terms)]
                logits = [t * (DH ** -0.5) for t in logits]
                if j == 0:
                    pos = jax.lax.broadcasted_iota(jnp.int32, (16, LANES), 1) + i * (BT * LANES)
                    logits = [jnp.where(pos >= DIL * w, t, -1e9) for w, t in enumerate(logits)]
                top = functools.reduce(jnp.maximum, logits)
                e = [jnp.exp(t - top) for t in logits]
                inv = 1.0 / functools.reduce(jnp.add, e)
                prob.append([t * inv for t in e])
            rows = [functools.reduce(jnp.add, [a * b for a, b in zip(prob[r // DH], window(1, j, r))])
                    for r in range(2 * DH)]
            heads.append(jnp.concatenate(rows, 0).astype(bf16))
        for m in range(2):
            kv_words[m, 0] = kv_words[m, BT]
        attn_inputs(jnp.minimum(i + 1, NB - 1))
        for j in range(BT):
            x = xs[i * BT + j].astype(f32)
            ys[i * BT + j] = project("o", "oR oP oQ", heads[j])[0] + x

    def glu_coeffs(i):
        for j in range(BT):
            ln[j, 0], ln[j, 1] = _layernorm_coeffs(lambda r: ys[i * BT + j, r:r + 16, :], 0.5)

    def gated(z, c):
        g, u = z[32 * c:32 * c + 16], z[32 * c + 16:32 * c + 32]
        return u * jnp.tanh(g) + u

    def glu_block(i, last):
        t0 = i * BT
        x = {r: [ys[t0 + j, r:r + 16, :] * ln[j, 0] - ln[j, 1] for j in range(BT)] for r in range(0, D, 16)}
        glu_coeffs(jnp.minimum(i + 1, NB - 1))
        x_ops = [_operands(_rhs_terms, [x[r], x[128 + r], x[256 + r], x[k3 + r]])
                 for k3, lo in ((384, 0), (448, 64)) for r in range(lo, 128, 16)]
        x_ops = [[jnp.concatenate([t[a][b] for t in x_ops], 0).astype(bf16) for b in range(7)] for a in range(7)]
        x_tail = jnp.concatenate([jnp.concatenate(x[r], 1) for r in range(448, D, 16)], 0).astype(bf16)
        early = [_dot(_load(wr, n), x_tail) for n in range(2)]
        h_ops = []
        for n in range(NP):
            shared = early[n] if n < len(early) else _dot(_load(wr, n), x_tail)
            init = [[shared[128 * b:128 * b + 128, LANES * j:LANES * j + LANES] for j in range(4)] for b in range(4)]
            for s in range(2):
                def up(a, b):
                    t = x_ops[a][b]
                    return _dot(_load(wp, n, s, a, b), jnp.concatenate([t[0:64], t[64 + 64 * s:128 + 64 * s]], 0))
                z = _strassen(up, init, _UP_ORDER)
                h = [[jnp.concatenate([gated(t[j], c) for t in z], 0) for j in range(4)] for c in range(4)]
                h_ops.append([[v.astype(bf16) for v in terms] for terms in _operands(_rhs_terms, h)])

        def down(a, b):
            return _dot(jnp.concatenate([_load(wd, n, a, b) for n in range(NP)], 1),
                        jnp.concatenate([t[a][b] for t in h_ops], 0))
        init = [[ys[t0 + j, QD * b:QD * b + QD, :] for j in range(4)] for b in range(4)]
        out = _strassen(down, init, _DOWN_ORDER)
        for j in range(BT):
            for b in ((2, 3, 0, 1) if j < 2 else (0, 1, 2, 3)):
                xs[t0 + j, QD * b:QD * b + QD, :] = out[b][j].astype(bf16)
            if j % 2:
                @pl.when(last)
                def _():
                    o_copy(t0 + j - 1).start()
                    o_copy(t0 + j).start()

    for n in range(3):
        start_wave(n)

    def clear_kv(j, _):
        kv[:, j] = jnp.zeros((2, D, LANES), bf16)
    jax.lax.fori_loop(0, BT + 1, clear_kv, None)
    jax.lax.fori_loop(0, 5, transpose_qkv, None)
    jax.lax.fori_loop(0, 3, reorder_qkv, None)
    wo_copy.wait()
    prepare_wo()
    for t in range(BT):
        x_copy(t).wait()

    def layer(l, _):
        attn_inputs(0)

        def attn_step(i, _):
            for step, (lo, hi) in enumerate(((BT, 2 * BT), (2 * BT, NT))):
                @pl.when((l == 0) & (i == step))
                def _():
                    jax.lax.fori_loop(lo, hi, lambda t, _: x_copy(t).wait(), None)
                    start_wave(8 + step)
            attn_block(i)

        jax.lax.fori_loop(0, NB, attn_step, None)
        pl.when(l == 0)(lambda: jax.lax.fori_loop(0, NP, prepare_glu, None))
        glu_coeffs(0)
        jax.lax.fori_loop(0, NB, lambda i, _: glu_block(i, l == 1), None)

    jax.lax.fori_loop(0, 2, layer, None)
    for t in range(NT):
        o_copy(t).wait()


@jax.jit
def pallas_interleave_layers__sliding_local_dilated__glu_gated_glu__prompt_kernel(
    A_x: jax.Array,
    A_wqkv: jax.Array,
    A_wo: jax.Array,
    B_x: jax.Array,
    B_w_gate: jax.Array,
    B_w_up: jax.Array,
    B_w_down: jax.Array,
):
    del B_x
    hbm = pl.BlockSpec(memory_space=pltpu.HBM)
    out = pl.pallas_call(
        _kernel,
        out_shape=jax.ShapeDtypeStruct((D, S), bf16),
        in_specs=[hbm] * 6,
        out_specs=hbm,
        scratch_shapes=[
            pltpu.VMEM((NT, D, LANES), bf16),
            pltpu.VMEM((NT, D, LANES), f32),
            pltpu.VMEM((D, 3 * D), bf16),
            pltpu.VMEM((D, D), bf16),
            pltpu.VMEM((NP, D, FP), bf16),
            pltpu.VMEM((NP, D, FP), bf16),
            pltpu.VMEM((NP, D, FP), bf16),
            pltpu.VMEM((5, 3 * D + 24, LANES), f32),
            pltpu.VMEM((4, 9, HD, LANES), bf16),
            pltpu.VMEM((NP, 2, 7, 7, 128, LANES), bf16),
            pltpu.VMEM((NP, 512, LANES), bf16),
            pltpu.VMEM((NP, 7, 7, QD, LANES), bf16),
            pltpu.VMEM((2, BT + 1, D, LANES), bf16),
            pltpu.VMEM((BT, D, LANES), bf16),
            pltpu.VMEM((BT, 2, 16, LANES), f32),
            pltpu.SemaphoreType.DMA((NT,)),
            pltpu.SemaphoreType.DMA((6,)),
            pltpu.SemaphoreType.DMA((3 * NP,)),
            pltpu.SemaphoreType.DMA((NT,)),
        ],
        compiler_params=pltpu.CompilerParams(vmem_limit_bytes=120 * 2**20),
    )(A_x.reshape(S, D).T, A_wqkv, A_wo, B_w_gate, B_w_up, B_w_down.T)
    return out.T.reshape(1, S, D)
```
